```python
import os as _os
_os.environ.setdefault("JAX_PLATFORMS", "cpu")
import jax
import jax.numpy as jnp

def _softmax(x, axis=-1):
    return jax.nn.softmax(x, axis=axis)
def _gelu(x):
    return jax.nn.gelu(x, approximate=True)
def _silu(x):
    return jax.nn.silu(x)
def _sigmoid(x):
    return jax.nn.sigmoid(x)
def _layernorm(x, axis=-1, eps=1e-5):
    m = jnp.mean(x, axis=axis, keepdims=True)
    v = jnp.var(x, axis=axis, keepdims=True)
    return (x - m) / jnp.sqrt(v + eps)
def _scatter_add(tgt, idx, src, axis=0):
    return tgt.at[idx].add(src)
def _segment_sum(src, seg, n):
    return jax.ops.segment_sum(src, seg, n)
class _Rng:
    def __init__(self, key):
        self._k = key
    def _next(self):
        self._k, sub = jax.random.split(self._k)
        return sub
    def normal(self, shape):
        return jax.random.normal(self._next(), shape, dtype=jnp.bfloat16)
    def randint(self, lo, hi, shape):
        return jax.random.randint(self._next(), shape, lo, hi, dtype=jnp.int32)
    def uniform(self, shape, lo=0.0, hi=1.0):
        return jax.random.uniform(self._next(), shape, jnp.bfloat16, lo, hi)
    def permutation(self, n):
        return jax.random.permutation(self._next(), n)


kernel_name = 'sequential_preLN__softmax_full_mha__dense_activation_squared_relu__prompt'

def setup_inputs():
    _rng = _Rng(jax.random.key(int.from_bytes(__import__("os").urandom(4), "little")))
    _w = (lambda a: (lambda t: t.astype(jnp.bfloat16) if jnp.issubdtype(t.dtype, jnp.floating) else t)(jnp.asarray(a)))
    def _A_setup():
        B, S, D = 1, 2048, 448
        return {
            "x": _w((lambda *s: _rng.normal(s) * 0.05)(B, S, D)),
            "wqkv": _w((lambda *s: _rng.normal(s) * 0.05)(D, 3 * D)),
            "wo": _w((lambda *s: _rng.normal(s) * 0.05)(D, D)),
        }
    _A_in = _A_setup()

    def _B_setup():
        B, S, D, F = 1, 2048, 448, 1792
        return {
            "x": _w((lambda *s: _rng.normal(s) * 0.05)(B, S, D)),
            "w1": _w((lambda *s: _rng.normal(s) * 0.05)(D, F)),
            "b1": _w((lambda *s: _rng.normal(s) * 0.05)(F)),
            "w2": _w((lambda *s: _rng.normal(s) * 0.05)(F, D)),
            "b2": _w((lambda *s: _rng.normal(s) * 0.05)(D)),
        }
    _B_in = _B_setup()

    return {
        "A_x": _A_in["x"],
        "A_wqkv": _A_in["wqkv"],
        "A_wo": _A_in["wo"],
        "B_x": _B_in["x"],
        "B_w1": _B_in["w1"],
        "B_b1": _B_in["b1"],
        "B_w2": _B_in["w2"],
        "B_b2": _B_in["b2"],
    }

def reference(A_x, A_wqkv, A_wo, B_x, B_w1, B_b1, B_w2, B_b2):
    def _A_ref(x, wqkv, wo):
        B, S, D = x.shape
        H = 16; Dh = D // H
        qkv = (lambda x, *d: x.transpose(*d))((x @ wqkv).reshape(B, S, 3, H, Dh), 2, 0, 3, 1, 4)
        q, k, v = qkv[0], qkv[1], qkv[2]
        scale = Dh ** -0.5
        scores = jnp.einsum("bhqd,bhkd->bhqk", q, k) * scale
        p = _softmax(scores, axis=-1)
        o = jnp.einsum("bhqk,bhkd->bhqd", p, v)
        return (lambda x, *d: x.transpose(*d))(o, 0, 2, 1, 3).reshape(B, S, D) @ wo

    def _B_ref(x, w1, b1, w2, b2):
        h = jnp.einsum("bsd,df->bsf", x, w1) + b1
        zero = jnp.zeros_like(h)
        r = jnp.where(h > zero, h, zero)
        h = r * r
        out = jnp.einsum("bsf,fd->bsd", h, w2) + b2
        return out

    x = A_x
    h = x + _A_ref(_layernorm(x, axis=-1), A_wqkv, A_wo)
    h2 = h + _B_ref(_layernorm(h, axis=-1), B_w1, B_b1, B_w2, B_b2)
    return h2
```

```python
import functools
import math

import jax
import jax.numpy as jnp
import jax.experimental.pallas as pl
import jax.experimental.pallas.tpu as pltpu

S = 2048
D = 448
DP = 512
H = 16
DH = 28
F = 1792
HP = 32
GW = 112
NG = 4
TQ = 256
NQ = S // TQ
CK = 256
NC = S // CK
LAG = 2
NBUF = 4
NTAIL = 4
NPRE = 1
CH = 256
NCH = S // CH
FC = 256
NF = F // FC
EPS = 1e-5
QSCALE = (DH ** -0.5) * math.log2(math.e)
f32 = jnp.float32
bf16 = jnp.bfloat16


def _ln_t(x):
    m = jnp.mean(x, axis=0, keepdims=True)
    xc = x - m
    v = jnp.mean(xc * xc, axis=0, keepdims=True)
    return xc * jax.lax.rsqrt(v + EPS)


def _kernel(xt_hbm, wqkv_hbm, wo_hbm, w1_hbm, b1_ref, w2t_hbm, b2_ref, o_ref,
            xt_ref, wqkv_ref, wo_ref, w1_ref, w2t_ref, sems,
            wqkt_scr, wvt_scr, wot_scr, w1t_scr, b2c_scr, qt_scr, k_scr, vt_scr,
            s0, s1, s2, s3, m_scr, ot_scr, z_ref):
    i = pl.program_id(0)
    bufs = (s0, s1, s2, s3)
    sub = jax.lax.broadcasted_iota(jnp.int32, (128, TQ), 0)

    def make_qk(tile, h, mfin):
        r0 = tile * TQ if isinstance(tile, int) else pl.multiple_of(tile * TQ, TQ)
        g, jj = divmod(h, NG)
        st = {}

        def qk(c):
            if c == 0:
                qg = qt_scr[GW * g:GW * g + 128, pl.ds(r0, TQ)]
                sel = (sub >= DH * jj) & (sub < DH * (jj + 1))
                st['q'] = jnp.where(sel, qg, jnp.zeros_like(qg))
            s = jnp.dot(k_scr[c * CK:(c + 1) * CK, 128 * g:128 * (g + 1)], st['q'],
                        preferred_element_type=f32)
            bufs[h % NBUF][c * CK:(c + 1) * CK, :] = s
            mc = jnp.max(s.reshape(CK // 8, 8, TQ), axis=0)
            st['m'] = mc if c == 0 else jnp.maximum(st['m'], mc)
            if c == NC - 1:
                m = jnp.max(st['m'], axis=0, keepdims=True)
                if mfin is None:
                    m_scr[...] = jnp.broadcast_to(m, m_scr.shape)
                else:
                    mfin[h] = m
        return qk

    @pl.when(i == 0)
    def _():
        cp_wqkv = pltpu.make_async_copy(wqkv_hbm, wqkv_ref, sems.at[0])
        cp_x = [pltpu.make_async_copy(xt_hbm.at[:, c * CH:(c + 1) * CH], xt_ref.at[:, c * CH:(c + 1) * CH],
                                      sems.at[4 + c]) for c in range(NCH)]
        cp_wo = pltpu.make_async_copy(wo_hbm, wo_ref, sems.at[1])
        cp_w1 = pltpu.make_async_copy(w1_hbm, w1_ref, sems.at[2])
        cp_w2 = pltpu.make_async_copy(w2t_hbm, w2t_ref, sems.at[3])
        cp_x[0].start()
        cp_wqkv.start()
        for c in range(1, NCH):
            cp_x[c].start()
        cp_wo.start()
        cp_w1.start()
        cp_w2.start()

        z_ref[0] = 0
        qt_scr[D:D + 16, :] = jnp.zeros((16, S), bf16)
        b2c_scr[...] = jnp.broadcast_to(b2_ref[...].astype(f32), (128, D)).T

        def ln_chunk(c):
            return _ln_t(xt_ref[:, c * CH:(c + 1) * CH].astype(f32)).astype(bf16)

        cp_x[0].wait()
        xn = {0: ln_chunk(0)}
        cp_wqkv.wait()
        cp_x[1].wait()
        wqkt_scr[...] = wqkv_ref[:, 0:1024].astype(f32).T.astype(bf16)
        wvt = wqkv_ref[:, 2 * D:3 * D].astype(f32).T
        zpad = jnp.zeros((HP - DH, D), f32)
        wvt_scr[...] = jnp.concatenate(
            [t for h in range(H) for t in (wvt[DH * h:DH * (h + 1), :], zpad)], axis=0).astype(bf16)
        row = jax.lax.broadcasted_iota(jnp.int32, (H * HP, CH), 0)
        ones_row = (row % HP) == DH

        def prep_wo():
            wot_scr[...] = wo_ref[...].astype(f32).T.astype(bf16)

        def prep_w1(c):
            rowd = jax.lax.broadcasted_iota(jnp.int32, (DP - D, FC), 0)
            b1c = b1_ref[:, c * FC:(c + 1) * FC].astype(f32)
            b1row = jnp.where(rowd == 0, jnp.broadcast_to(b1c, (DP - D, FC)), 0.0)
            w1aug = jnp.concatenate([w1_ref[:, c * FC:(c + 1) * FC].astype(f32), b1row], axis=0)
            w1t_scr[c * FC:(c + 1) * FC, :] = w1aug.T.astype(bf16)

        preps = [prep_wo] + [functools.partial(prep_w1, c) for c in range(NF)]
        for c in range(NCH):
            r = c * CH
            if c == 1:
                for cc in range(2, NCH):
                    cp_x[cc].wait()
            if c == 4:
                cp_wo.wait()
                cp_w1.wait()
                cp_w2.wait()
            if c + 1 < NCH:
                xn[c + 1] = ln_chunk(c + 1)
            if c >= 4:
                for t in preps[2 * (c - 4):2 * (c - 3)]:
                    t()
            qt = jnp.dot(wqkt_scr[0:D, :], xn[c], preferred_element_type=f32)
            qt_scr[0:D, r:r + CH] = (qt * QSCALE).astype(bf16)
            kt = jnp.dot(wqkt_scr[D:2 * D + 16, :], xn[c], preferred_element_type=f32)
            kt = kt.astype(bf16).astype(f32)
            for g in range(NG):
                k_scr[r:r + CH, 128 * g:128 * (g + 1)] = kt[GW * g:GW * g + 128, :].T.astype(bf16)
            vt = jnp.dot(wvt_scr[...], xn[c], preferred_element_type=f32)
            vt_scr[:, r:r + CH] = jnp.where(ones_row, 1.0, vt).astype(bf16)

        qk0 = make_qk(0, 0, None)
        for c in range(NC):
            qk0(c)

    z = pl.multiple_of(z_ref[0], 8)
    r0 = pl.multiple_of(i * TQ, TQ)
    mfin = [None] * H
    mfin[0] = m_scr[0:1, :]
    acc = [None] * H
    qks = [None] + [make_qk(i, h, mfin) for h in range(1, H)]
    qk_next = make_qk(jnp.minimum(i + 1, NQ - 1), 0, None)

    def pv(j):
        h, c = divmod(j, NC)
        p = jnp.exp2(bufs[h % NBUF][pl.ds(z + c * CK, CK), :] - mfin[h]).astype(bf16)
        o = jnp.dot(vt_scr[HP * h:HP * (h + 1), c * CK:(c + 1) * CK], p, preferred_element_type=f32)
        acc[h] = o if acc[h] is None else acc[h] + o
        if c == NC - 1:
            a = acc[h]
            ot_scr[DH * h:DH * (h + 1), :] = a[0:DH, :] / a[DH:DH + 1, :]

    st = {}

    def outproj():
        attn = jnp.dot(wot_scr[...], ot_scr[...].astype(bf16), preferred_element_type=f32)
        h1 = xt_ref[:, pl.ds(r0, TQ)].astype(f32) + attn
        rowp = jax.lax.broadcasted_iota(jnp.int32, (DP - D, TQ), 0)
        st['hn'] = jnp.concatenate([_ln_t(h1), jnp.where(rowp == 0, 1.0, 0.0)], axis=0).astype(bf16)
        b2c = b2c_scr[...]
        st['y'] = h1 + jnp.concatenate([b2c] * (TQ // 128), axis=1)

    def up(c):
        u = jnp.dot(w1t_scr[c * FC:(c + 1) * FC, :], st['hn'], preferred_element_type=f32)
        u = jnp.maximum(u, 0.0)
        st['u', c] = (u * u).astype(bf16)

    def down(c):
        st['y'] = st['y'] + jnp.dot(w2t_ref[:, c * FC:(c + 1) * FC], st['u', c],
                                    preferred_element_type=f32)

    T = H * NC
    TQK = (H - 1) * NC
    for j in range(TQK):
        qks[1 + j // NC](j % NC)
        if j >= LAG:
            pv(j - LAG)
    nxt = 0
    for n, j in enumerate(range(TQK - LAG, T)):
        if n % 2 == 0 and nxt < NTAIL:
            qk_next(nxt)
            nxt += 1
        pv(j)
    for _ in range(NPRE):
        qk_next(nxt)
        nxt += 1
    outproj()
    while nxt < NC:
        qk_next(nxt)
        nxt += 1
    up(0)
    for c in range(NF):
        if c + 1 < NF:
            up(c + 1)
        down(c)
    o_ref[...] = st['y'].astype(o_ref.dtype)


@jax.jit
def pallas_sequential_preLN__softmax_full_mha__dense_activation_squared_relu__prompt_kernel(
    A_x, A_wqkv, A_wo, B_x, B_w1, B_b1, B_w2, B_b2):
    xt = A_x.reshape(S, D).T
    full = lambda shape: pl.BlockSpec(shape, lambda i: (0,) * len(shape))
    hbm = pl.BlockSpec(memory_space=pl.ANY)
    out = pl.pallas_call(
        _kernel,
        grid=(NQ,),
        in_specs=[hbm, hbm, hbm, hbm, full((1, F)), hbm, full((1, D))],
        out_specs=pl.BlockSpec((D, TQ), lambda i: (0, i)),
        out_shape=jax.ShapeDtypeStruct((D, S), A_x.dtype),
        scratch_shapes=[
            pltpu.VMEM((D, S), bf16), pltpu.VMEM((D, 3 * D), bf16), pltpu.VMEM((D, D), bf16),
            pltpu.VMEM((D, F), bf16), pltpu.VMEM((D, F), bf16), pltpu.SemaphoreType.DMA((4 + NCH,)),
            pltpu.VMEM((1024, D), bf16), pltpu.VMEM((H * HP, D), bf16), pltpu.VMEM((D, D), bf16),
            pltpu.VMEM((F, DP), bf16), pltpu.VMEM((D, 128), f32),
            pltpu.VMEM((D + 16, S), bf16), pltpu.VMEM((S, 512), bf16), pltpu.VMEM((H * HP, S), bf16),
            pltpu.VMEM((S, TQ), f32), pltpu.VMEM((S, TQ), f32), pltpu.VMEM((S, TQ), f32), pltpu.VMEM((S, TQ), f32),
            pltpu.VMEM((8, TQ), f32),
            pltpu.VMEM((D, TQ), f32), pltpu.SMEM((1,), jnp.int32),
        ],
        compiler_params=pltpu.CompilerParams(
            dimension_semantics=("arbitrary",), vmem_limit_bytes=100 * 1024 * 1024),
    )(xt, A_wqkv, A_wo, B_w1, B_b1.reshape(1, F), B_w2.T, B_b2.reshape(1, D))
    return out.T.reshape(A_x.shape)
```

```python
import functools
import math

import jax
import jax.numpy as jnp
import jax.experimental.pallas as pl
import jax.experimental.pallas.tpu as pltpu

S = 2048
D = 448
DP = 512
H = 16
DH = 28
F = 1792
HP = 32
GW = 112
NG = 4
TQ = 256
NQ = S // TQ
CK = 256
NC = S // CK
LAG = 2
NBUF = 4
NTAIL = 4
NPRE = 1
CH = 256
NCH = S // CH
FC = 256
NF = F // FC
EPS = 1e-5
QSCALE = (DH ** -0.5) * math.log2(math.e)
f32 = jnp.float32
bf16 = jnp.bfloat16


def _ln_t(x):
    m = jnp.mean(x, axis=0, keepdims=True)
    xc = x - m
    v = jnp.mean(xc * xc, axis=0, keepdims=True)
    return xc * jax.lax.rsqrt(v + EPS)


def _kernel(xt_hbm, wqkv_hbm, wo_hbm, w1_hbm, b1_hbm, w2t_hbm, b2_hbm, o_ref,
            xt_ref, wqkv_ref, wo_ref, w1_ref, w2t_ref, sems,
            wqkt_scr, wot_scr, w1t_scr, b2c_scr, qt_scr, k_scr, vt_scr,
            s0, s1, s2, s3, m_scr, ot_scr, z_ref, b1_ref, b2_ref):
    i = pl.program_id(0)
    bufs = (s0, s1, s2, s3)
    sub = jax.lax.broadcasted_iota(jnp.int32, (128, TQ), 0)

    def make_qk(tile, h, mfin):
        r0 = tile * TQ if isinstance(tile, int) else pl.multiple_of(tile * TQ, TQ)
        g, jj = divmod(h, NG)
        st = {}

        def qk(c):
            if c == 0:
                qg = qt_scr[GW * g:GW * g + 128, pl.ds(r0, TQ)]
                sel = (sub >= DH * jj) & (sub < DH * (jj + 1))
                st['q'] = jnp.where(sel, qg, jnp.zeros_like(qg))
            s = jnp.dot(k_scr[c * CK:(c + 1) * CK, 128 * g:128 * (g + 1)], st['q'],
                        preferred_element_type=f32)
            bufs[h % NBUF][c * CK:(c + 1) * CK, :] = s
            mc = jnp.max(s.reshape(CK // 8, 8, TQ), axis=0)
            st['m'] = mc if c == 0 else jnp.maximum(st['m'], mc)
            if c == NC - 1:
                m = jnp.max(st['m'], axis=0, keepdims=True)
                if mfin is None:
                    m_scr[...] = jnp.broadcast_to(m, m_scr.shape)
                else:
                    mfin[h] = m
        return qk

    @pl.when(i == 0)
    def _():
        wsl = ((0, 512), (512, 1024), (1024, 3 * D))
        cp_wqkv = [pltpu.make_async_copy(wqkv_hbm.at[:, a:b], wqkv_ref.at[:, a:b], sems.at[n])
                   for n, (a, b) in enumerate(wsl)]
        cp_x = [pltpu.make_async_copy(xt_hbm.at[:, c * CH:(c + 1) * CH], xt_ref.at[:, c * CH:(c + 1) * CH],
                                      sems.at[8 + c]) for c in range(NCH)]
        cp_wo = pltpu.make_async_copy(wo_hbm, wo_ref, sems.at[3])
        cp_w1 = pltpu.make_async_copy(w1_hbm, w1_ref, sems.at[4])
        cp_w2 = pltpu.make_async_copy(w2t_hbm, w2t_ref, sems.at[5])
        cp_b1 = pltpu.make_async_copy(b1_hbm, b1_ref, sems.at[6])
        cp_b2 = pltpu.make_async_copy(b2_hbm, b2_ref, sems.at[7])
        cp_x[0].start()
        for cp in cp_wqkv:
            cp.start()
        for c in range(1, NCH):
            cp_x[c].start()
        cp_b1.start()
        cp_b2.start()
        cp_wo.start()
        cp_w1.start()
        cp_w2.start()

        z_ref[0] = 0
        qt_scr[D:D + 16, :] = jnp.zeros((16, S), bf16)

        def ln_chunk(c):
            return _ln_t(xt_ref[:, c * CH:(c + 1) * CH].astype(f32)).astype(bf16)

        def wt(a, b):
            wqkt_scr[a:b, :] = wqkv_ref[:, a:b].astype(f32).T.astype(bf16)

        cp_x[0].wait()
        xn = {0: ln_chunk(0)}
        cp_wqkv[0].wait()
        wt(0, 512)
        st0 = {}
        row8 = jax.lax.broadcasted_iota(jnp.int32, (8, CH), 0)
        one4 = jnp.where(row8 == 4, 1.0, 0.0)
        one0 = jnp.where(row8 == 0, 1.0, 0.0)

        def prep_wo():
            wot_scr[...] = wo_ref[...].astype(f32).T.astype(bf16)

        def prep_w1(c):
            rowd = jax.lax.broadcasted_iota(jnp.int32, (DP - D, FC), 0)
            b1c = st0['b1'][:, c * FC:(c + 1) * FC]
            b1row = jnp.where(rowd == 0, jnp.broadcast_to(b1c, (DP - D, FC)), 0.0)
            w1aug = jnp.concatenate([w1_ref[:, c * FC:(c + 1) * FC].astype(f32), b1row], axis=0)
            w1t_scr[c * FC:(c + 1) * FC, :] = w1aug.T.astype(bf16)

        preps = [prep_wo] + [functools.partial(prep_w1, c) for c in range(NF)]
        for c in range(NCH):
            r = c * CH
            if c == 1:
                for cc in range(2, NCH):
                    cp_x[cc].wait()
            if c == 4:
                cp_b1.wait()
                cp_b2.wait()
                cp_wo.wait()
                cp_w1.wait()
                cp_w2.wait()
                b2c_scr[...] = jnp.broadcast_to(b2_ref[...].astype(f32).reshape(1, D), (128, D)).T
                st0['b1'] = b1_ref[...].astype(f32).reshape(1, F)
            if 0 < c < NCH - 1:
                xn[c + 1] = ln_chunk(c + 1)
            if c >= 4:
                for t in preps[2 * (c - 4):2 * (c - 3)]:
                    t()
            qt = jnp.dot(wqkt_scr[0:D, :], xn[c], preferred_element_type=f32)
            qt_scr[0:D, r:r + CH] = (qt * QSCALE).astype(bf16)
            if c == 0:
                cp_wqkv[1].wait()
                cp_wqkv[2].wait()
                cp_x[1].wait()
                wt(512, 1280)
                wt(1280, 3 * D)
                xn[1] = ln_chunk(1)
            kvt = jnp.dot(wqkt_scr[D:3 * D, :], xn[c], preferred_element_type=f32)
            kt = kvt[0:D + 16, :].astype(bf16).astype(f32)
            for g in range(NG):
                k_scr[r:r + CH, 128 * g:128 * (g + 1)] = kt[GW * g:GW * g + 128, :].T.astype(bf16)
            parts = []
            for j in range(H // 2):
                b = D + 2 * DH * j
                mid = kvt[b + 24:b + 32, :]
                parts += [kvt[b:b + 24, :], jnp.where(row8 < 4, mid, one4),
                          jnp.where(row8 >= 4, mid, one0), kvt[b + 32:b + 56, :]]
            vt_scr[:, r:r + CH] = jnp.concatenate(parts, axis=0).astype(bf16)

        qk0 = make_qk(0, 0, None)
        for c in range(NC):
            qk0(c)

    z = pl.multiple_of(z_ref[0], 8)
    r0 = pl.multiple_of(i * TQ, TQ)
    mfin = [None] * H
    mfin[0] = m_scr[0:1, :]
    acc = [None] * H
    qks = [None] + [make_qk(i, h, mfin) for h in range(1, H)]
    qk_next = make_qk(jnp.minimum(i + 1, NQ - 1), 0, None)

    def pv(j):
        h, c = divmod(j, NC)
        p = jnp.exp2(bufs[h % NBUF][pl.ds(z + c * CK, CK), :] - mfin[h]).astype(bf16)
        o = jnp.dot(vt_scr[HP * h:HP * (h + 1), c * CK:(c + 1) * CK], p, preferred_element_type=f32)
        acc[h] = o if acc[h] is None else acc[h] + o
        if c == NC - 1:
            a = acc[h]
            if h % 2 == 0:
                ot_scr[DH * h:DH * (h + 1), :] = a[0:DH, :] / a[DH:DH + 1, :]
            else:
                ot_scr[DH * h:DH * (h + 1), :] = (a / a[0:1, :])[HP - DH:HP, :]

    st = {}

    def outproj():
        attn = jnp.dot(wot_scr[...], ot_scr[...].astype(bf16), preferred_element_type=f32)
        h1 = xt_ref[:, pl.ds(r0, TQ)].astype(f32) + attn
        rowp = jax.lax.broadcasted_iota(jnp.int32, (DP - D, TQ), 0)
        st['hn'] = jnp.concatenate([_ln_t(h1), jnp.where(rowp == 0, 1.0, 0.0)], axis=0).astype(bf16)
        b2c = b2c_scr[...]
        st['y'] = h1 + jnp.concatenate([b2c] * (TQ // 128), axis=1)

    def up(c):
        u = jnp.dot(w1t_scr[c * FC:(c + 1) * FC, :], st['hn'], preferred_element_type=f32)
        u = jnp.maximum(u, 0.0)
        st['u', c] = (u * u).astype(bf16)

    def down(c):
        st['y'] = st['y'] + jnp.dot(w2t_ref[:, c * FC:(c + 1) * FC], st['u', c],
                                    preferred_element_type=f32)

    T = H * NC
    TQK = (H - 1) * NC
    for j in range(TQK):
        qks[1 + j // NC](j % NC)
        if j >= LAG:
            pv(j - LAG)
    nxt = 0
    for n, j in enumerate(range(TQK - LAG, T)):
        if n % 2 == 0 and nxt < NTAIL:
            qk_next(nxt)
            nxt += 1
        pv(j)
    for _ in range(NPRE):
        qk_next(nxt)
        nxt += 1
    outproj()
    while nxt < NC:
        qk_next(nxt)
        nxt += 1
    up(0)
    for c in range(NF):
        if c + 1 < NF:
            up(c + 1)
        down(c)
    o_ref[...] = st['y'].astype(o_ref.dtype)


@jax.jit
def pallas_sequential_preLN__softmax_full_mha__dense_activation_squared_relu__prompt_kernel(
    A_x, A_wqkv, A_wo, B_x, B_w1, B_b1, B_w2, B_b2):
    xt = A_x.reshape(S, D).T
    hbm = pl.BlockSpec(memory_space=pl.ANY)
    out = pl.pallas_call(
        _kernel,
        grid=(NQ,),
        in_specs=[hbm] * 7,
        out_specs=pl.BlockSpec((D, TQ), lambda i: (0, i)),
        out_shape=jax.ShapeDtypeStruct((D, S), A_x.dtype),
        scratch_shapes=[
            pltpu.VMEM((D, S), bf16), pltpu.VMEM((D, 3 * D), bf16), pltpu.VMEM((D, D), bf16),
            pltpu.VMEM((D, F), bf16), pltpu.VMEM((D, F), bf16),
            pltpu.SemaphoreType.DMA((8 + NCH,)),
            pltpu.VMEM((3 * D, D), bf16), pltpu.VMEM((D, D), bf16),
            pltpu.VMEM((F, DP), bf16), pltpu.VMEM((D, 128), f32),
            pltpu.VMEM((D + 16, S), bf16), pltpu.VMEM((S, 512), bf16), pltpu.VMEM((H * HP, S), bf16),
            pltpu.VMEM((S, TQ), f32), pltpu.VMEM((S, TQ), f32), pltpu.VMEM((S, TQ), f32), pltpu.VMEM((S, TQ), f32),
            pltpu.VMEM((8, TQ), f32),
            pltpu.VMEM((D, TQ), f32), pltpu.SMEM((1,), jnp.int32),
            pltpu.VMEM((F,), bf16), pltpu.VMEM((D,), bf16),
        ],
        compiler_params=pltpu.CompilerParams(
            dimension_semantics=("arbitrary",), vmem_limit_bytes=100 * 1024 * 1024),
    )(xt, A_wqkv, A_wo, B_w1, B_b1, B_w2.T, B_b2)
    return out.T.reshape(A_x.shape)
```

```python
import functools
import math

import jax
import jax.numpy as jnp
import jax.experimental.pallas as pl
import jax.experimental.pallas.tpu as pltpu

S = 2048
D = 448
DP = 512
H = 16
DH = 28
F = 1792
HP = 32
GW = 112
NG = 4
TQ = 256
NQ = S // TQ
CK = 128
NC = S // CK
LAG = 4
NBUF = 4
NTAIL = 8
NPRE = 2
CH = 256
NCH = S // CH
FC = 256
NF = F // FC
HA, HB = 14, 15
NV = {HA: 12, HB: 10}
NHM = 14
NPC = CK // 8
TA, TB = 20, 180
AOP = 8
NCP = 2
TOKD = 4
QW = [2] * 8 + [4] * 3 + [6, 6, 6, 5, 5]
AUP = (10,) * NF
ADN = (8, 8, 8, 8, 8, 7, 3)
GENS_PER_CHUNK = (0, 48, 48, 48, 38, 38, 38, 38, 12)
VR = 2 * DH
EPS = 1e-5
QSCALE = (DH ** -0.5) * math.log2(math.e)
f32 = jnp.float32
bf16 = jnp.bfloat16
u32 = jnp.uint32


def _ln_t(x):
    m = jnp.mean(x, axis=0, keepdims=True)
    xc = x - m
    v = jnp.mean(xc * xc, axis=0, keepdims=True)
    return xc * jax.lax.rsqrt(v + EPS)


def _schedule():
    qk = [('qk', h, c) for h in (HA, HB) for c in range(NV[h], NC)]
    qk += [('qk', h, c) for h in range(1, NHM) for c in range(NC)]
    main = [('pv', h, c) for h in range(NHM) for c in range(NC)]
    extra = {}
    for c in range(NC):
        extra.setdefault(TA + c, []).append(('pv', HA, c))
        extra.setdefault(TB + 2 * c, []).append(('pv', HB, c))
    items = []
    mi = 0
    done = {0: -LAG - 1}
    for j, it in enumerate(qk):
        items.append(it + (2 if j % 2 == 0 else 0,))
        if it[2] == NC - 1:
            done[it[1]] = j
        h = main[mi][1]
        if j >= LAG and h in done and j > done[h] + LAG:
            items.append(main[mi] + (0,))
            mi += 1
        items += [e + (0,) for e in extra.pop(j, [])]
    assert not extra
    nxt = 0
    for n, it in enumerate(main[mi:]):
        if n % 4 < 2 and nxt < NTAIL:
            items.append(('qn', 0, nxt, 1 if nxt % 2 == 0 else 0))
            nxt += 1
        items.append(it + (0,))
    for _ in range(NPRE):
        items.append(('qn', 0, nxt, 2 if nxt % 2 == 0 else 0))
        nxt += 1
    items.append(('op', 0, 0, AOP))
    while nxt < NC:
        items.append(('qn', 0, nxt, 0))
        nxt += 1
    items.append(('up', 0, 0, AUP[0]))
    for c in range(NF):
        if c + 1 < NF:
            items.append(('up', 0, c + 1, AUP[c + 1]))
        items.append(('dn', 0, c, ADN[c]))
    return items


ITEMS = _schedule()
PIECES = ([(HA, NV[HA] - 1, j, 0) for j in range(NPC)]
          + [(HB, c, j, 0) for c in range(NV[HB]) for j in range(NPC)]
          + [(HA, c, j, 1) for c in range(NV[HA] - 1) for j in range(NPC)])
assert sum(it[3] for it in ITEMS) == len(PIECES), (sum(it[3] for it in ITEMS), len(PIECES))
GENS = [(h, c, d) for c in range(NCH) for h in (HA, HB) if 2 * c < NV[h] for d in range(DH)]
assert sum(GENS_PER_CHUNK) == len(GENS), len(GENS)
KPR = VR * (max(NV.values()) // 2)


def _kernel(xt_hbm, wqkv_hbm, wo_hbm, w1_hbm, b1_hbm, w2t_hbm, b2_hbm, o_ref,
            xt_ref, wqkv_ref, wo_ref, w1_ref, w2t_ref, sems,
            wqkt_scr, wot_scr, w1t_scr, b2c_scr, qt_scr, k_scr, vt_scr,
            s0, s1, s2, s3, sa_scr, sb_scr, m_scr, mp_scr, ot_scr,
            qtv_scr, kp_scr, kba_scr, kbb_scr, qr_scrs, z_ref, b1_ref, b2_ref):
    i = pl.program_id(0)
    bufs = (s0, s1, s2, s3)
    kbs = {HA: kba_scr, HB: kbb_scr}
    qrs = {HA: qr_scrs[:NCP], HB: qr_scrs[NCP:]}
    sub = jax.lax.broadcasted_iota(jnp.int32, (128, TQ), 0)

    def sbuf(h):
        return sa_scr if h == HA else sb_scr if h == HB else bufs[0 if h == 0 else 1 + (h - 1) % (NBUF - 1)]

    def col0(tile):
        return tile * TQ if isinstance(tile, int) else pl.multiple_of(tile * TQ, TQ)

    def make_qk(tile, h, last, fin, side):
        g, jj = divmod(h, NG)
        st = {}

        def qk(c, na):
            if 'q' not in st:
                qg = qt_scr[GW * g:GW * g + 128, pl.ds(col0(tile), TQ)]
                sel = (sub >= DH * jj) & (sub < DH * (jj + 1))
                st['q'] = jnp.where(sel, qg, jnp.zeros_like(qg))
            s = jnp.dot(k_scr[c * CK:(c + 1) * CK, 128 * g:128 * (g + 1)], st['q'],
                        preferred_element_type=f32)
            sbuf(h)[c * CK:(c + 1) * CK, :] = s
            if na:
                s = side(s, na, QW)
            mb = jnp.max(s.reshape(CK // 8, 8, TQ), axis=0)
            st['m'] = mb if 'm' not in st else jnp.maximum(st['m'], mb)
            if c == last:
                fin(st['m'])
        return qk

    def fin_next(m):
        m_scr[...] = jnp.broadcast_to(jnp.max(m, axis=0, keepdims=True), m_scr.shape)

    def copy_q(h, tile):
        lo, hi = (0, 32) if h == HA else (24, VR)
        q = qtv_scr[lo:hi, pl.ds(col0(tile), TQ)]
        for qr in qrs[h]:
            qr[lo:hi, :] = q

    @pl.when(i == 0)
    def _():
        wsl = ((0, 512), (512, 1024), (1024, 3 * D))
        cp_wqkv = [pltpu.make_async_copy(wqkv_hbm.at[:, a:b], wqkv_ref.at[:, a:b], sems.at[n])
                   for n, (a, b) in enumerate(wsl)]
        cp_x = [pltpu.make_async_copy(xt_hbm.at[:, c * CH:(c + 1) * CH], xt_ref.at[:, c * CH:(c + 1) * CH],
                                      sems.at[8 + c]) for c in range(NCH)]
        cp_wo = pltpu.make_async_copy(wo_hbm, wo_ref, sems.at[3])
        cp_w1 = pltpu.make_async_copy(w1_hbm, w1_ref, sems.at[4])
        cp_w2 = pltpu.make_async_copy(w2t_hbm, w2t_ref, sems.at[5])
        cp_b1 = pltpu.make_async_copy(b1_hbm, b1_ref, sems.at[6])
        cp_b2 = pltpu.make_async_copy(b2_hbm, b2_ref, sems.at[7])
        cp_x[0].start()
        for cp in cp_wqkv:
            cp.start()
        for c in range(1, NCH):
            cp_x[c].start()
        cp_b1.start()
        cp_b2.start()
        cp_wo.start()
        cp_w1.start()
        cp_w2.start()

        z_ref[0] = 0
        z0 = pl.multiple_of(i * 8, 8)
        qt_scr[D:D + 16, :] = jnp.zeros((16, S), bf16)

        def ln_chunk(c):
            return _ln_t(xt_ref[:, c * CH:(c + 1) * CH].astype(f32)).astype(bf16)

        def wt(a, b):
            wqkt_scr[a:b, :] = wqkv_ref[:, a:b].astype(f32).T.astype(bf16)

        cp_x[0].wait()
        xn = {0: ln_chunk(0)}
        cp_wqkv[0].wait()
        wt(0, 512)
        st0 = {'g': 0}
        row8 = jax.lax.broadcasted_iota(jnp.int32, (8, CH), 0)
        one4 = jnp.where(row8 == 4, 1.0, 0.0)
        one0 = jnp.where(row8 == 0, 1.0, 0.0)

        def prep_wo():
            wot_scr[...] = wo_ref[...].astype(f32).T.astype(bf16)

        def prep_w1(c):
            rowd = jax.lax.broadcasted_iota(jnp.int32, (DP - D, FC), 0)
            b1c = st0['b1'][:, c * FC:(c + 1) * FC]
            b1row = jnp.where(rowd == 0, jnp.broadcast_to(b1c, (DP - D, FC)), 0.0)
            w1aug = jnp.concatenate([w1_ref[:, c * FC:(c + 1) * FC].astype(f32), b1row], axis=0)
            w1t_scr[c * FC:(c + 1) * FC, :] = w1aug.T.astype(bf16)

        def gen(which, tok):
            h, c, d = GENS[st0['g']]
            st0['g'] += 1
            kp_scr[pl.ds(z0 + KPR, 8), :] = pltpu.bitcast(tok, u32)
            r = VR * c + DH * (h - HA) + d
            t = jnp.broadcast_to(kp_scr[r:r + 1, :], (128, 128)).T
            lo = pltpu.bitcast(t << 16, f32)
            hi = pltpu.bitcast(t & jnp.uint32(0xFFFF0000), f32)
            kbs[h][2 * c * NPC:(2 * c + 1) * NPC, d] = lo.reshape(NPC, 8, 128)
            kbs[h][(2 * c + 1) * NPC:(2 * c + 2) * NPC, d] = hi.reshape(NPC, 8, 128)

        def gens(x, n):
            R = x.shape[0] // 8
            for k in range(n):
                half, r = divmod(k * 2 * R // n, R)
                gen(0, x[8 * r:8 * r + 8, 128 * half:128 * (half + 1)])

        preps = [prep_wo] + [functools.partial(prep_w1, c) for c in range(NF)]
        for c in range(NCH):
            r = c * CH
            if c == 1:
                for cc in range(2, NCH):
                    cp_x[cc].wait()
            if c == 4:
                cp_b1.wait()
                cp_b2.wait()
                cp_wo.wait()
                cp_w1.wait()
                cp_w2.wait()
                b2c_scr[...] = jnp.broadcast_to(b2_ref[...].astype(f32).reshape(1, D), (128, D)).T
                st0['b1'] = b1_ref[...].astype(f32).reshape(1, F)
            if 0 < c < NCH - 1:
                xn[c + 1] = ln_chunk(c + 1)
            if c >= 4:
                for t in preps[2 * (c - 4):2 * (c - 3)]:
                    t()
            ng = GENS_PER_CHUNK[c]
            qt = jnp.dot(wqkt_scr[0:D, :], xn[c], preferred_element_type=f32)
            gens(qt, ng // 3)
            qt = (qt * QSCALE).astype(bf16)
            qt_scr[0:D, r:r + CH] = qt
            qtv_scr[:, r:r + CH] = qt.astype(f32)[DH * HA:D, :]
            if c == 0:
                cp_wqkv[1].wait()
                cp_wqkv[2].wait()
                cp_x[1].wait()
                wt(512, 1280)
                wt(1280, 3 * D)
                xn[1] = ln_chunk(1)
            kvt = jnp.dot(wqkt_scr[D:3 * D, :], xn[c], preferred_element_type=f32)
            gens(kvt, ng - ng // 3)
            kt = kvt[0:D + 16, :].astype(bf16).astype(f32)
            if VR * c < KPR:
                kv = pltpu.bitcast(kt[DH * HA:D, :], u32)
                kp_scr[VR * c:VR * (c + 1), :] = kv[:, 128:] | (kv[:, :128] >> 16)
            for g in range(NG):
                k_scr[r:r + CH, 128 * g:128 * (g + 1)] = kt[GW * g:GW * g + 128, :].T.astype(bf16)
            parts = []
            for j in range(H // 2):
                b = D + 2 * DH * j
                mid = kvt[b + 24:b + 32, :]
                parts += [kvt[b:b + 24, :], jnp.where(row8 < 4, mid, one4),
                          jnp.where(row8 >= 4, mid, one0), kvt[b + 32:b + 56, :]]
            vt_scr[:, r:r + CH] = jnp.concatenate(parts, axis=0).astype(bf16)

        def fin_part(m):
            mp_scr[...] = m

        def gen1(x, na, w):
            gen(0, x[0:8, 0:128])
            return x

        copy_q(HA, 0)
        qka = make_qk(0, HA, NV[HA] - 2, fin_part, gen1)
        for c in range(NV[HA] - 1):
            qka(c, 1 if st0['g'] < len(GENS) else 0)
        qk0 = make_qk(0, 0, NC - 1, fin_next, gen1)
        for c in range(NC):
            qk0(c, 1 if st0['g'] < len(GENS) else 0)
        assert st0['g'] == len(GENS)

    z = pl.multiple_of(z_ref[0], 8)
    r0 = col0(i)
    nxt = jnp.minimum(i + 1, NQ - 1)
    mfin = {0: m_scr[0:1, :]}
    mpart = {}
    mv = {(HA, 0): mp_scr[...]}
    acc = [None] * H
    copy_q(HB, i)
    vp = {'n': 0}
    never = jax.lax.broadcasted_iota(jnp.int32, (8, 128), 0) + z < 0

    def link(x, a):
        return jnp.concatenate([jnp.where(never, a[:, n0:n0 + 128], x[:, n0:n0 + 128])
                                for n0 in range(0, TQ, 128)], axis=1)

    def release(x, n):
        for k in range(vp['n'], vp['n'] + n):
            pi, d = divmod(k, DH)
            h, c, j, nx = PIECES[pi]
            if d == TOKD and pi + 1 < len(PIECES):
                h2, c2, j2, nx2 = PIECES[pi + 1]
                if nx2 and c2 == 0 and j2 == 0:
                    copy_q(h2, nxt)
                qrs[h2][(pi + 1) % NCP][pl.ds(z + VR, 8), 0:128] = x[:, 0:128]
            r = DH * (h - HA) + d
            kb = kbs[h][c * NPC + j, d]
            t = jnp.concatenate([kb * jnp.broadcast_to(qrs[h][pi % NCP][r:r + 1, n0:n0 + 128], (8, 128))
                                 for n0 in range(0, TQ, 128)], axis=1)
            a = vp['a'] = t if d == 0 else vp['a'] + t
            if d == DH - 1:
                sbuf(h)[c * CK + 8 * j:c * CK + 8 * j + 8, :] = a
                mv[h, nx] = a if (h, nx) not in mv else jnp.maximum(mv[h, nx], a)
            if d == DH - 1 or k == vp['n'] + n - 1:
                x = link(x, a)
        vp['n'] += n
        return x

    def side(x, na, w):
        R = x.shape[0] // 8
        w = [w[g * len(w) // R] for g in range(R)]
        tot = int(round(na * DH))
        cum = 0
        parts = []
        for g in range(R):
            n = (cum + w[g]) * tot // sum(w) - cum * tot // sum(w)
            cum += w[g]
            parts.append(release(x[8 * g:8 * g + 8], n))
        return jnp.concatenate(parts, axis=0)

    def fin_h(h, m):
        if h in NV:
            mpart[h] = m
        else:
            mfin[h] = jnp.max(m, axis=0, keepdims=True)

    qks = {h: make_qk(i, h, NC - 1, functools.partial(fin_h, h), side) for h in range(1, H)}
    qk_next = make_qk(nxt, 0, NC - 1, fin_next, side)

    def pv(h, c):
        if h not in mfin:
            mfin[h] = jnp.max(jnp.maximum(mv[h, 0], mpart[h]), axis=0, keepdims=True)
        p = jnp.exp2(sbuf(h)[pl.ds(z + c * CK, CK), :] - mfin[h]).astype(bf16)
        o = jnp.dot(vt_scr[HP * h:HP * (h + 1), c * CK:(c + 1) * CK], p, preferred_element_type=f32)
        acc[h] = o if acc[h] is None else acc[h] + o
        if c == NC - 1:
            a = acc[h]
            if h % 2 == 0:
                ot_scr[DH * h:DH * (h + 1), :] = a[0:DH, :] / a[DH:DH + 1, :]
            else:
                ot_scr[DH * h:DH * (h + 1), :] = (a / a[0:1, :])[HP - DH:HP, :]

    st = {}

    def side_sum(p, q, na, w):
        x = side(jnp.concatenate([p, q], axis=1), na, w)
        return x[:, :128] + x[:, 128:]

    def dot_halves(w_ref, rows, x, na, ws):
        out = []
        for n in range(2):
            pq = [jnp.dot(w_ref[rows, a:b], x[a:b, 128 * n:128 * (n + 1)], preferred_element_type=f32)
                  for a, b in ((0, 256), (256, x.shape[0]))]
            out.append(side_sum(*pq, na / 2, ws[n]))
        return jnp.concatenate(out, axis=1)

    def outproj(na):
        attn = dot_halves(wot_scr, slice(0, D), ot_scr[...].astype(bf16), na,
                          ([1, 0] * 28, [1, 0] * 24 + [0] * 8))
        h1 = xt_ref[:, pl.ds(r0, TQ)].astype(f32) + attn
        rowp = jax.lax.broadcasted_iota(jnp.int32, (DP - D, TQ), 0)
        st['hn'] = jnp.concatenate([_ln_t(h1), jnp.where(rowp == 0, 1.0, 0.0)], axis=0).astype(bf16)
        b2c = b2c_scr[...]
        st['y'] = h1 + jnp.concatenate([b2c] * (TQ // 128), axis=1)

    def up(c, na):
        u = dot_halves(w1t_scr, slice(c * FC, (c + 1) * FC), st['hn'], na, ([1], [1]))
        u = jnp.maximum(u, 0.0)
        st['u', c] = (u * u).astype(bf16)

    def down(c, na):
        y = jnp.dot(w2t_ref[:, c * FC:(c + 1) * FC], st['u', c], preferred_element_type=f32)
        y0 = side_sum(y[:, :128], st['y'][:, :128], na, [1, 0] if c == NF - 1 else [1])
        st['y'] = jnp.concatenate([y0, st['y'][:, 128:] + y[:, 128:]], axis=1)

    for kind, a, b, na in ITEMS:
        if kind == 'qk':
            qks[a](b, na)
        elif kind == 'qn':
            qk_next(b, na)
        elif kind == 'pv':
            pv(a, b)
        elif kind == 'op':
            outproj(na)
        elif kind == 'up':
            up(b, na)
        else:
            down(b, na)
    assert vp['n'] == DH * len(PIECES)
    mp_scr[...] = mv[HA, 1]
    o_ref[...] = st['y'].astype(o_ref.dtype)


@jax.jit
def pallas_sequential_preLN__softmax_full_mha__dense_activation_squared_relu__prompt_kernel(
    A_x, A_wqkv, A_wo, B_x, B_w1, B_b1, B_w2, B_b2):
    xt = A_x.reshape(S, D).T
    hbm = pl.BlockSpec(memory_space=pl.ANY)
    sbuf = pltpu.VMEM((S, TQ), f32)
    out = pl.pallas_call(
        _kernel,
        grid=(NQ,),
        in_specs=[hbm] * 7,
        out_specs=pl.BlockSpec((D, TQ), lambda i: (0, i)),
        out_shape=jax.ShapeDtypeStruct((D, S), A_x.dtype),
        scratch_shapes=[
            pltpu.VMEM((D, S), bf16), pltpu.VMEM((D, 3 * D), bf16), pltpu.VMEM((D, D), bf16),
            pltpu.VMEM((D, F), bf16), pltpu.VMEM((D, F), bf16),
            pltpu.SemaphoreType.DMA((8 + NCH,)),
            pltpu.VMEM((3 * D, D), bf16), pltpu.VMEM((D, D), bf16),
            pltpu.VMEM((F, DP), bf16), pltpu.VMEM((D, 128), f32),
            pltpu.VMEM((D + 16, S), bf16), pltpu.VMEM((S, 512), bf16), pltpu.VMEM((H * HP, S), bf16),
            sbuf, sbuf, sbuf, sbuf, sbuf, sbuf,
            pltpu.VMEM((8, TQ), f32), pltpu.VMEM((8, TQ), f32),
            pltpu.VMEM((D, TQ), f32),
            pltpu.VMEM((VR, S), f32), pltpu.VMEM((KPR + 8, 128), u32),
            pltpu.VMEM((NV[HA] * NPC, DH, 8, 128), f32), pltpu.VMEM((NV[HB] * NPC, DH, 8, 128), f32),
            [pltpu.VMEM((VR + 8, TQ), f32)] * (2 * NCP),
            pltpu.SMEM((1,), jnp.int32),
            pltpu.VMEM((F,), bf16), pltpu.VMEM((D,), bf16),
        ],
        compiler_params=pltpu.CompilerParams(
            dimension_semantics=("arbitrary",), vmem_limit_bytes=110 * 1024 * 1024),
    )(xt, A_wqkv, A_wo, B_w1, B_b1, B_w2.T, B_b2)
    return out.T.reshape(A_x.shape)
```

```python
import functools
import math

import jax
import jax.numpy as jnp
import jax.experimental.pallas as pl
import jax.experimental.pallas.tpu as pltpu

S = 2048
D = 448
DP = 512
H = 16
DH = 28
F = 1792
HP = 32
GW = 112
NG = 4
G0 = (0, GW, 2 * GW, D - 128)
TQ = 256
NQ = S // TQ
CK = 128
NC = S // CK
LAG = 4
NBUF = 4
NTAIL = 12
NPRE = 2
TAILN = (1, 1, 2, 2, 2, 2, 1, 1, 2, 2, 2, 2)
CH = 256
NCH = S // CH
FC = 256
NF = F // FC
HA, HB = 14, 15
NV = {HA: 16, HB: 12}
NPC = CK // 8
CL = 7
XP = (2, 6, 10, 16, 166, 170, 174, 178, 182, 186, 192, 196)
MH = (1, 2, 3, 4, 6, 7, 8, 9, 10, 11, 12, 13, 5)
KB = 9
HIM = 6
NCP = 2
TOKD = 4
PE, PO = (2, 6, 9, 10, 12, 13, 15), (12, 13, 15)
PFIRST = {0: (0, 0)}
PLOW, PHIGH = ((2, 6, 10, 13, 15), (12, 13, 15)), ((2, 4, 6, 9, 10, 12, 13, 15), (10, 12, 13, 15))
PAT = {j: PLOW for j in list(range(0, 24)) + list(range(158, 198))}
PAT.update({j: ((6, 10, 13, 15), (13, 15)) for j in range(2, 18)})
PAT.update({j: PHIGH for j in range(44, 140) if (j - 12) % 16 < 12})
PTAIL = (2, 5, 8, 11, 14)
PLAST = ((4, 10, 12, 14, 15), (9, 11, 13, 14, 15))
COP = (44, 20)
SKIP = (180, 194)
LNGAP = ((2, 3), (3, 5))
NXB = 5
GPD = ([(0, 1), (0, 1), (18, 1), (21, 1), (18, .8), (0, 1), (19, 1), (21, 1), (21, 1), (21, 1), (17, 1)]
       + [(13, .6)] + [(16, 1), (15, 1), (16, 1)] * 2 + [(18, 1)] * 6)
OSPLIT = (0, 128, 256, 368, D)
NO = len(OSPLIT) - 1
NPOS = 2 * D // 8
VR = 2 * DH
EPS = 1e-5
QSCALE = (DH ** -0.5) * math.log2(math.e)
f32 = jnp.float32
bf16 = jnp.bfloat16
u32 = jnp.uint32


def _pack(x):
    return pltpu.bitcast(x.astype(bf16), u32)


def _unpack(x):
    return pltpu.bitcast(x, bf16)


def _even(n, R):
    return tuple(int((k + 0.5) * R / n) for k in range(n))


PIECES1 = ([(HB, c, j, 0) for c in range(NV[HB]) for j in range(NPC)]
           + [(HA, c, j, 1) for c in range(NV[HA]) for j in range(NPC)])


def _schedule():
    qk = [('qk', h, c) for h in (HA, HB) for c in range(NV[h], NC)]
    qk += [('qk', h, c) for h in MH for c in range(NC)]
    order = (0, HA) + MH[:KB] + (HB,) + MH[KB:]
    main = [('pv', h, c) for h in order for c in range(NC)]
    extra = [1] + [t + c for t in XP for c in range(2)]
    items = []
    mi = 0
    done = {0: -LAG - 1, HA: -LAG - 1}
    for j, it in enumerate(qk):
        items.append(it + (PFIRST.get(j, ()) + PAT.get(j, (PE, PO))[j % 2],))
        if it[2] == NC - 1:
            done[it[1]] = j
        for _ in range((j >= 1) + (j in extra)):
            _, h, c = main[mi]
            assert j > done[h] + LAG, (j, h, c)
            if h == HB and c == 0:
                n = sum(len(x[3]) for x in items) * CL // DH
                assert n > max([k for k, pc in enumerate(PIECES1) if pc[0] == h and not pc[3]]) + 2, n
            items.append(main[mi] + ((),))
            mi += 1
    assert sum(TAILN) == len(main) - mi and len(TAILN) == NTAIL
    for nxt, n in enumerate(TAILN):
        mid = PTAIL if nxt % 2 == 0 else PO if nxt > 2 else ()
        items.append(('qn', 0, nxt, PLAST[nxt % 2] if nxt >= NTAIL - 2 else mid))
        items += [it + ((),) for it in main[mi:mi + n]]
        mi += n
    nxt = NTAIL
    for _ in range(NPRE):
        items.append(('qn', 0, nxt, PE if nxt % 2 == 0 else PO))
        nxt += 1
    items.append(('op', 0, 0, _even(COP[0], 56) + tuple(56 + g for g in _even(COP[1], 44))))
    while nxt < NC:
        items.append(('qn', 0, nxt, ()))
        nxt += 1
    ffn = [('up', 0, 0)]
    for c in range(NF - 1):
        ffn += [('up', 1, c), ('up', 0, c + 1)] + [('up', 1, c + 1)] * (c == NF - 2) + [('dn', 0, c)]
    ffn += [('dn', 0, NF - 1)]
    n = sum(len(x[3]) for x in items)
    n1 = -(-n * CL // DH // 2) * 2
    pieces = [p + (1,) for p in PIECES1[:n1]] + [p + (2,) for p in PIECES1[n1::2]]
    left = len(pieces) * DH // CL - n
    size = [32 if it[0] == 'up' else 56 for it in ffn]
    lo, hi = 16, sum(size) - HIM
    ok = [g for g in range(lo, hi) if not SKIP[0] <= sum(size) - g < SKIP[1]]
    pos = [ok[g] for g in _even(left, len(ok))]
    base = 0
    for it, n in zip(ffn, size):
        items.append(it + (tuple(g - base for g in pos if base <= g < base + n),))
        base += n
    return items, pieces


ITEMS, PIECES = _schedule()
GENS = [(h, c, d) for c in range(NCH) for h in (HA, HB) if 2 * c < NV[h] for d in range(DH)]
KPR = VR * (max(NV.values()) // 2)


def _kernel(xt_hbm, wqkv_hbm, wo_hbm, w1_hbm, b1_hbm, w2t_hbm, b2_hbm, o_hbm,
            xt_ref, wqkv_ref, wo_ref, w1_ref, w2t_ref, sems, osems, ob_scr,
            wqkt_scr, wot_scr, w1t_scr, b2c_scr, xn_scr, qt_scr, k_scr, vt_scr,
            s0, s1, s2, s3, sa_scr, sb_scr, m_scr, mp_scr, ot_scr,
            qtv_scr, kp_scr, kba_scr, kbb_scr, qr_scrs, z_ref, b1_ref, b2_ref):
    i = pl.program_id(0)
    bufs = (s0, s1, s2, s3)
    kbs = {HA: kba_scr, HB: kbb_scr}
    qrs = {HA: qr_scrs[:NCP], HB: qr_scrs[NCP:]}
    sub = jax.lax.broadcasted_iota(jnp.int32, (64, TQ), 0)

    def sbuf(h):
        return sa_scr if h == HA else sb_scr if h == HB else bufs[0 if h == 0 else 1 + MH.index(h) % (NBUF - 1)]

    def col0(tile):
        return tile * TQ if isinstance(tile, int) else pl.multiple_of(tile * TQ, TQ)

    def make_qk(tile, h, last, fin, side):
        g = h // NG
        st = {}

        def qk(c, na):
            if 'q' not in st:
                qg = qt_scr[G0[g] // 2:G0[g] // 2 + 64, pl.ds(col0(tile), TQ)]
                lo = (DH * h - G0[g]) // 2
                sel = (sub >= lo) & (sub < lo + DH // 2)
                st['q'] = _unpack(jnp.where(sel, qg, jnp.zeros_like(qg)))
            s = jnp.dot(_unpack(k_scr[c * CK // 2:(c + 1) * CK // 2, 128 * g:128 * (g + 1)]), st['q'],
                        preferred_element_type=f32)
            sbuf(h)[c * CK:(c + 1) * CK, :] = s
            s = side(s, na)
            mb = jnp.max(s.reshape(CK // 8, 8, TQ), axis=0)
            st['m'] = mb if 'm' not in st else jnp.maximum(st['m'], mb)
            if c == last:
                fin(st['m'])
        return qk

    def fin_next(m, ref=m_scr):
        ref[...] = jnp.broadcast_to(jnp.max(m, axis=0, keepdims=True), ref.shape)

    def copy_q(h, tile):
        lo, hi = (0, 32) if h == HA else (24, VR)
        q = qtv_scr[lo:hi, pl.ds(col0(tile), TQ)]
        for qr in qrs[h]:
            qr[lo:hi, :] = q

    @pl.when(i == 0)
    def _():
        wsl = ((384, 640), (640, 2 * D), (0, 384), (2 * D, 3 * D))
        cp_wqkv = [pltpu.make_async_copy(wqkv_hbm.at[:, a:b], wqkv_ref.at[:, a:b], sems.at[n])
                   for n, (a, b) in zip((0, 1, 2, 8 + NCH), wsl)]
        cp_x = [pltpu.make_async_copy(xt_hbm.at[:, c * CH:(c + 1) * CH], xt_ref.at[:, c * CH:(c + 1) * CH],
                                      sems.at[8 + c]) for c in range(NCH)]
        cp_wo = pltpu.make_async_copy(wo_hbm, wo_ref, sems.at[3])
        cp_w1 = pltpu.make_async_copy(w1_hbm, w1_ref, sems.at[4])
        cp_w2 = pltpu.make_async_copy(w2t_hbm, w2t_ref, sems.at[5])
        cp_b1 = pltpu.make_async_copy(b1_hbm, b1_ref, sems.at[6])
        cp_b2 = pltpu.make_async_copy(b2_hbm, b2_ref, sems.at[7])
        cp_x[0].start()
        cp_wqkv[0].start()
        cp_wqkv[1].start()
        cp_x[1].start()
        cp_wqkv[2].start()
        cp_x[2].start()
        cp_wqkv[3].start()
        for c in range(3, NCH):
            cp_x[c].start()
        cp_b1.start()
        cp_b2.start()
        cp_wo.start()
        cp_w1.start()
        cp_w2.start()

        z_ref[0] = 0
        z0 = pl.multiple_of(i * 8, 8)

        def ln_steps(c):
            t = {}

            def x(k, r0, r1):
                return xt_ref[r0:r1, pl.ds(pl.multiple_of(i * (k * CH) + c * CH, CH), CH)].astype(f32)

            def add(key, v):
                v = jnp.sum(v.reshape(v.shape[0] // 8, 8, CH), axis=0)
                t[key] = v if key not in t else t[key] + v
                return t[key]

            def s1(r):
                return add('s', x(0, r, r + 32))

            def s2(r):
                if r == 0:
                    t['m'] = jnp.sum(t['s'], axis=0, keepdims=True) * (1.0 / D)
                xc = x(1, r, r + 32) - t['m']
                return add('v', xc * xc)

            def s3(r):
                if r == 0:
                    t['r'] = jax.lax.rsqrt(jnp.sum(t['v'], axis=0, keepdims=True) * (1.0 / D) + EPS)
                y = _pack((x(2, r, r + 16) - t['m']) * t['r'])
                xn_scr[r // 2:r // 2 + 8, c * CH:(c + 1) * CH] = y
                return jax.lax.bitcast_convert_type(y, f32)

            return ([functools.partial(s1, r) for r in range(0, D, 32)]
                    + [functools.partial(s2, r) for r in range(0, D, 32)]
                    + [functools.partial(s3, r) for r in range(0, D, 16)])

        def wt(a, b):
            wqkt_scr[a // 2:b // 2, :] = _pack(wqkv_ref[:, a:b].astype(f32).T)

        never0 = jax.lax.broadcasted_iota(jnp.int32, (8, CH), 0) + z0 < 0
        plan = {}
        st0 = {'g': 0, 'dot': 0, 'late': [], 'k': []}
        row8 = jax.lax.broadcasted_iota(jnp.int32, (8, CH), 0)
        one4 = jnp.where(row8 == 4, 1.0, 0.0)
        one0 = jnp.where(row8 == 0, 1.0, 0.0)

        def prep_wo():
            wot_scr[...] = _pack(wo_ref[...].astype(f32).T)

        def prep_w1(c):
            rowd = jax.lax.broadcasted_iota(jnp.int32, (DP - D, FC), 0)
            b1c = st0['b1'][:, c * FC:(c + 1) * FC]
            b1row = jnp.where(rowd == 0, jnp.broadcast_to(b1c, (DP - D, FC)), 0.0)
            w1aug = jnp.concatenate([w1_ref[:, c * FC:(c + 1) * FC].astype(f32), b1row], axis=0)
            w1t_scr[c * FC // 2:(c + 1) * FC // 2, :] = _pack(w1aug.T)

        def gen(tok):
            h, c, d = GENS[st0['g']]
            assert c in st0['k']
            st0['g'] += 1
            kp_scr[pl.ds(z0 + KPR, 8), :] = jax.lax.bitcast_convert_type(tok, u32)
            r = VR * c + DH * (h - HA) + d
            t = jnp.broadcast_to(kp_scr[r:r + 1, :], (128, 128)).T
            lo = jax.lax.bitcast_convert_type(t << 16, f32)
            hi = jax.lax.bitcast_convert_type(t & jnp.uint32(0xFFFF0000), f32)
            kbs[h][2 * c * NPC:(2 * c + 1) * NPC, d] = lo.reshape(NPC, 8, 128)
            kbs[h][(2 * c + 1) * NPC:(2 * c + 2) * NPC, d] = hi.reshape(NPC, 8, 128)
            st0['late'].append(jnp.concatenate([lo[120:], hi[120:]], axis=1))

        def spread(steps, dot0, ndots):
            for k, f in enumerate(steps):
                plan.setdefault(int((dot0 + (k + 0.5) * ndots / len(steps)) * NPOS), []).append(f)

        def proj(c, part):
            rows = slice(part * D // 2, (part + 1) * D // 2)
            n, frac = GPD[st0['dot']]
            toks = [int(k * NPOS * frac / n) for k in range(n)]
            pos = st0['dot'] * NPOS
            st0['dot'] += 1
            out = []
            for half in range(2):
                if half:
                    st0.pop('mid', lambda: None)()
                cols = slice(c * CH + 128 * half, c * CH + 128 * (half + 1))
                x = jnp.concatenate(
                    [jnp.dot(_unpack(wqkt_scr[rows, a:b]), _unpack(xn_scr[a // 2:b // 2, cols]),
                             preferred_element_type=f32) for a, b in ((0, 256), (256, D))], axis=1)
                parts = []
                for g in range(D // 8):
                    xg = x[8 * g:8 * g + 8]
                    if half * (D // 8) + g in toks:
                        gen(xg[:, 0:128])
                    for f in plan.pop(pos + half * (D // 8) + g, []):
                        xg = jnp.where(never0, f(), xg)
                    parts.append(xg[:, :128] + xg[:, 128:])
                out.append(jnp.concatenate(parts, axis=0))
            return jnp.concatenate(out, axis=1)

        def proj_q(c):
            qt = (proj(c, 0) * QSCALE).astype(bf16)
            qt_scr[:, c * CH:(c + 1) * CH] = _pack(qt)
            qtv_scr[:, c * CH:(c + 1) * CH] = qt.astype(f32)[DH * HA:D, :]

        def proj_k(c):
            kt = proj(c, 1).astype(bf16).astype(f32)
            st0['k'].append(c)
            if VR * c < KPR:
                kv = jax.lax.bitcast_convert_type(kt[DH * HA:D, :], u32)
                kp_scr[VR * c:VR * (c + 1), :] = kv[:, 128:] | (kv[:, :128] >> 16)
            for g in range(NG):
                k_scr[c * CH // 2:(c + 1) * CH // 2, 128 * g:128 * (g + 1)] = _pack(kt[G0[g]:G0[g] + 128, :].T)

        def proj_v(c):
            vt = proj(c, 2)
            parts = []
            for j in range(H // 2):
                b = 2 * DH * j
                mid = vt[b + 24:b + 32, :]
                parts += [vt[b:b + 24, :], jnp.where(row8 < 4, mid, one4),
                          jnp.where(row8 >= 4, mid, one0), vt[b + 32:b + 56, :]]
            vt_scr[:, c * CH:(c + 1) * CH] = _pack(jnp.concatenate(parts, axis=0))

        cp_x[0].wait()
        for f in ln_steps(0):
            f()
        for n in range(2):
            cp_wqkv[n].wait()
            wt(*wsl[n])

        def mid_x():
            cp_x[1].wait()
            for f in ln_steps(1):
                f()

        def mid_a():
            cp_wqkv[2].wait()
            cp_x[2].wait()
            wt(*wsl[2])

        def mid_b():
            cp_wqkv[3].wait()
            for cc in range(3, NXB):
                cp_x[cc].wait()
            wt(2 * D, 1280)
            wt(1280, 3 * D)

        st0['mid'] = mid_x
        proj_k(0)
        st0['mid'] = mid_a
        spread(ln_steps(2), 1.5, 2.1)
        proj_k(1)
        proj_q(0)
        proj_q(1)
        proj_k(2)
        st0['mid'] = mid_b
        spread(ln_steps(3), 5.5, 3)
        proj_q(2)
        for c in range(3):
            proj_v(c)
        preps = [prep_wo] + [functools.partial(prep_w1, c) for c in range(NF)]
        for c in range(3, NCH):
            if c == 4:
                for cc in range(NXB, NCH):
                    cp_x[cc].wait()
                cp_b1.wait()
                cp_b2.wait()
                cp_wo.wait()
                cp_w1.wait()
                b2c_scr[...] = jnp.broadcast_to(b2_ref[...].astype(f32).reshape(1, D), (128, D)).T
                st0['b1'] = b1_ref[...].astype(f32).reshape(1, F)
            if c < NCH - 1:
                spread(ln_steps(c + 1), 3 * c, 2.6)
            if c >= 4:
                for t in preps[2 * (c - 4):2 * (c - 3)]:
                    t()
            proj_k(c)
            proj_q(c)
            proj_v(c)

        def gen1(x, na):
            st0['dot'] += 1
            if st0['g'] < len(GENS):
                if st0['dot'] % 6 != 1:
                    gen(x[0:8, 0:128])
            elif na and st0['late']:
                return jnp.concatenate([jnp.where(never0, st0['late'].pop(0), x[0:8]), x[8:]], axis=0)
            return x

        qka = make_qk(0, HA, NV[HA] - 1, functools.partial(fin_next, ref=mp_scr), gen1)
        for c in range(NV[HA]):
            qka(c, 0)
        qk0 = make_qk(0, 0, NC - 1, fin_next, gen1)
        st0['late'] = st0['late'][-9:]
        for c in range(NC):
            qk0(c, c >= 4)
        assert st0['g'] == len(GENS) and not plan
        cp_w2.wait()

    def cp_out(t, k):
        rows = slice(OSPLIT[k], OSPLIT[k + 1])
        return pltpu.make_async_copy(ob_scr.at[t, rows], o_hbm.at[rows, pl.ds(col0(t), TQ)], osems.at[k, t])

    def step(i, carry):
        z = pl.multiple_of(z_ref[0], 8)
        r0 = col0(i)
        nxt = jnp.minimum(i + 1, NQ - 1)
        mfin = {0: m_scr[0:1, :], HA: mp_scr[0:1, :]}
        mv = {}
        acc = [None] * H
        copy_q(HB, i)
        vp = {'n': 0, 'steps': [], 'every': 1, 'skip': 0, 'left': False, 'pend': []}
        never = jax.lax.broadcasted_iota(jnp.int32, (8, 128), 0) + z < 0

        never2 = jax.lax.broadcasted_iota(jnp.int32, (8, 128), 1) + z < 0

        def link(x, a):
            if vp['left']:
                x0 = jnp.where(never2, a[:, 128:], jnp.where(never, a[:, :128], x[:, :128]))
                return jnp.concatenate([x0, x[:, 128:]], axis=1)
            return jnp.concatenate([jnp.where(never, a[:, n0:n0 + 128], x[:, n0:n0 + 128])
                                    for n0 in range(0, TQ, 128)], axis=1)

        def release(x, n):
            if vp['pend']:
                x = link(x, vp['pend'].pop())
            for k in range(vp['n'], vp['n'] + n):
                pi, d = divmod(k, DH)
                h, c, j, nx, w = PIECES[pi]
                if d == TOKD and NCP <= pi + 1 < len(PIECES):
                    h2, c2, j2, nx2, _ = PIECES[pi + 1]
                    if nx2 and c2 == 0 and j2 == 0:
                        copy_q(h2, nxt)
                    qrs[h2][(pi + 1) % NCP][pl.ds(z + VR, 8), 0:128] = x[:, 0:128]
                r = DH * (h - HA) + d
                qb = [jnp.broadcast_to(qrs[h][pi % NCP][r:r + 1, n0:n0 + 128], (8, 128)) for n0 in range(0, TQ, 128)]
                t = [jnp.concatenate([kbs[h][c * NPC + j + u, d] * q for q in qb], axis=1) for u in range(w)]
                a = vp['a'] = t if d == 0 else [a0 + t0 for a0, t0 in zip(vp['a'], t)]
                if d == DH - 1:
                    for u in range(w):
                        sbuf(h)[c * CK + 8 * (j + u):c * CK + 8 * (j + u + 1), :] = a[u]
                        mv[h, nx] = a[u] if (h, nx) not in mv else jnp.maximum(mv[h, nx], a[u])
                    if h == HB and PIECES[pi + 1][0] != HB:
                        mfin[h] = jnp.max(mv[h, 0], axis=0, keepdims=True)
                if d == DH - 1 or k == vp['n'] + n - 1:
                    x = link(x, a[0])
                    assert not vp['pend']
                    vp['pend'] = a[1:]
            vp['n'] += n
            return x

        def side(x, pos):
            parts = []
            for g in range(x.shape[0] // 8):
                xg = release(x[8 * g:8 * g + 8], CL * pos.count(g))
                if vp['skip']:
                    vp['skip'] -= 1
                elif vp['steps'] and g % vp['every'] == 0:
                    vp['steps'].pop(0)(x[8 * g:8 * g + 8, 128:])
                parts.append(xg)
            return jnp.concatenate(parts, axis=0)

        def fin_h(h, m):
            if h == HB:
                mv[h, 0] = jnp.maximum(mv[h, 0], m)
            else:
                mfin[h] = jnp.max(m, axis=0, keepdims=True)

        qks = {h: make_qk(i, h, NC - 1, functools.partial(fin_h, h), side) for h in range(1, H)}
        qk_next = make_qk(nxt, 0, NC - 1, fin_next, side)

        def pv(h, c):
            p = jnp.exp2(sbuf(h)[pl.ds(z + c * CK, CK), :] - mfin[h]).astype(bf16)
            o = jnp.dot(_unpack(vt_scr[HP // 2 * h:HP // 2 * (h + 1), c * CK:(c + 1) * CK]), p,
                        preferred_element_type=f32)
            acc[h] = o if acc[h] is None else acc[h] + o
            if c == NC - 1:
                a = acc[h]
                if h == MH[-1]:
                    st['ol'] = a / a[0:1, :]
                elif h % 2 == 0:
                    ot_scr[DH * h:DH * (h + 1), :] = a[0:DH, :] / a[DH:DH + 1, :]
                else:
                    ot_scr[DH * h:DH * (h + 1), :] = (a / a[0:1, :])[HP - DH:HP, :]

        st = {}

        def side_sum(p, q, pos):
            x = side(jnp.concatenate([p, q], axis=1), pos)
            return x[:, :128] + x[:, 128:]

        def halves(x):
            return x[:256].astype(bf16), x[256:].astype(bf16)

        def dot_half(w_ref, rows, xs, pos):
            pq = [jnp.dot(_unpack(w_ref[rows, a:a + x.shape[0]]), x, preferred_element_type=f32)
                  for a, x in zip((0, 256), xs)]
            vp['left'] = True
            out = side_sum(*pq, pos)
            vp['left'] = False
            return out

        def outproj(pos):
            for n in range(2):
                cols = slice(128 * n, 128 * (n + 1))
                e = DH * (MH[-1] + 1)
                low = jax.lax.broadcasted_iota(jnp.int32, (8, 128), 0) < HP - DH
                ot = jnp.concatenate([ot_scr[0:e - HP, cols],
                                      jnp.where(low, ot_scr[e - HP:e - HP + 8, cols], st['ol'][0:8, cols]),
                                      st['ol'][8:, cols], ot_scr[e:, cols]], axis=0)
                attn = dot_half(wot_scr, slice(0, D // 2), halves(ot),
                                tuple(g - 56 * n for g in pos))
                h1 = xt_ref[:, pl.ds(r0 + 128 * n, 128)].astype(f32) + attn
                st['y', n] = h1 + b2c_scr[...]
                m = jnp.broadcast_to(jnp.sum(h1, axis=0, keepdims=True) * (1.0 / D), (8, 128))
                h1 = h1.reshape(D // 64, 8, 8, 128)
                hn = []

                def var(k, gate, h1=h1, m=m, n=n):
                    xc = h1[k] - jnp.where(never, gate, m)
                    v = jnp.sum(xc * xc, axis=0)
                    st['v', n] = v if k == 0 else st['v', n] + v

                def norm(k, gate, h1=h1, m=m, n=n, hn=hn):
                    if k == 0:
                        rs = jax.lax.rsqrt(jnp.sum(st['v', n], axis=0, keepdims=True) * (1.0 / D) + EPS)
                        st['rs'] = jnp.broadcast_to(rs, (8, 128))
                        st['mrs'] = m * st['rs']
                    hn.append((h1[k] * jnp.where(never, gate, st['rs']) - st['mrs']).reshape(64, 128))
                    if k == D // 64 - 1:
                        rowp = jax.lax.broadcasted_iota(jnp.int32, (DP - D, 128), 0)
                        st['hn', n] = halves(jnp.concatenate(hn + [jnp.where(rowp == 0, 1.0, 0.0)], axis=0))

                nop = [lambda gate: None]
                vp['steps'] += (nop * LNGAP[n][0] + [functools.partial(var, k) for k in range(D // 64)]
                                + nop * LNGAP[n][1] + [functools.partial(norm, k) for k in range(D // 64)])
                vp['every'] = 1 if n else 2
                vp['skip'] = 16 if n else 0

        def up(n, c, pos):
            u = jnp.maximum(dot_half(w1t_scr, slice(c * FC // 2, (c + 1) * FC // 2), st['hn', n], pos), 0.0)
            st['u', c, n] = u * u

        def down(c, pos):
            u = jnp.concatenate([st['u', c, 0], st['u', c, 1]], axis=1).astype(bf16)
            y = jnp.dot(w2t_ref[:, c * FC:(c + 1) * FC], u, preferred_element_type=f32)
            if c >= NF - 2:
                y = side(y, pos)
                st['y', 0] = st['y', 0] + y[:, :128]
            else:
                st['y', 0] = side_sum(y[:, :128], st['y', 0], pos)
            st['y', 1] = st['y', 1] + y[:, 128:]

        for kind, a, b, na in ITEMS:
            if kind == 'qk':
                qks[a](b, na)
            elif kind == 'qn':
                qk_next(b, na)
            elif kind == 'pv':
                pv(a, b)
            elif kind == 'op':
                outproj(na)
            elif kind == 'up':
                up(a, b, na)
            else:
                down(b, na)
        assert vp['n'] == DH * len(PIECES) and not vp['pend']
        fin_next(mv[HA, 1], mp_scr)
        y = jnp.concatenate([st['y', 0], st['y', 1]], axis=1).astype(ob_scr.dtype)
        for k in range(NO):
            ob_scr[i, OSPLIT[k]:OSPLIT[k + 1]] = y[OSPLIT[k]:OSPLIT[k + 1]]
            cp_out(i, k).start()
        return carry

    @pl.when(i == 1)
    def _():
        jax.lax.fori_loop(0, NQ, step, 0)
        for t in range(NQ):
            for k in range(NO):
                cp_out(t, k).wait()


@jax.jit
def pallas_sequential_preLN__softmax_full_mha__dense_activation_squared_relu__prompt_kernel(
    A_x, A_wqkv, A_wo, B_x, B_w1, B_b1, B_w2, B_b2):
    xt = A_x.reshape(S, D).T
    hbm = pl.BlockSpec(memory_space=pl.ANY)
    sbuf = pltpu.VMEM((S, TQ), f32)
    out = pl.pallas_call(
        _kernel,
        grid=(2,),
        in_specs=[hbm] * 7,
        out_specs=hbm,
        out_shape=jax.ShapeDtypeStruct((D, S), A_x.dtype),
        scratch_shapes=[
            pltpu.VMEM((D, S), bf16), pltpu.VMEM((D, 3 * D), bf16), pltpu.VMEM((D, D), bf16),
            pltpu.VMEM((D, F), bf16), pltpu.VMEM((D, F), bf16),
            pltpu.SemaphoreType.DMA((9 + NCH,)), pltpu.SemaphoreType.DMA((NO, NQ)),
            pltpu.VMEM((NQ, D, TQ), A_x.dtype),
            pltpu.VMEM((3 * D // 2, D), u32), pltpu.VMEM((D // 2, D), u32),
            pltpu.VMEM((F // 2, DP), u32), pltpu.VMEM((D, 128), f32),
            pltpu.VMEM((D // 2, S), u32),
            pltpu.VMEM((D // 2, S), u32), pltpu.VMEM((S // 2, 512), u32), pltpu.VMEM((H * HP // 2, S), u32),
            sbuf, sbuf, sbuf, sbuf, sbuf, sbuf,
            pltpu.VMEM((8, TQ), f32), pltpu.VMEM((8, TQ), f32),
            pltpu.VMEM((D, TQ), f32),
            pltpu.VMEM((VR, S), f32), pltpu.VMEM((KPR + 8, 128), u32),
            pltpu.VMEM((NV[HA] * NPC, DH, 8, 128), f32), pltpu.VMEM((NV[HB] * NPC, DH, 8, 128), f32),
            [pltpu.VMEM((VR + 8, TQ), f32)] * (2 * NCP),
            pltpu.SMEM((1,), jnp.int32),
            pltpu.VMEM((F,), bf16), pltpu.VMEM((D,), bf16),
        ],
        compiler_params=pltpu.CompilerParams(
            dimension_semantics=("arbitrary",), vmem_limit_bytes=110 * 1024 * 1024,
            disable_bounds_checks=True, disable_semaphore_checks=True),
    )(xt, A_wqkv, A_wo, B_w1, B_b1, B_w2.T, B_b2)
    return out.T.reshape(A_x.shape)
```
